```python
import os as _os
_os.environ.setdefault("JAX_PLATFORMS", "cpu")
import jax
import jax.numpy as jnp

def _softmax(x, axis=-1):
    return jax.nn.softmax(x, axis=axis)
def _gelu(x):
    return jax.nn.gelu(x, approximate=True)
def _silu(x):
    return jax.nn.silu(x)
def _sigmoid(x):
    return jax.nn.sigmoid(x)
def _layernorm(x, axis=-1, eps=1e-5):
    m = jnp.mean(x, axis=axis, keepdims=True)
    v = jnp.var(x, axis=axis, keepdims=True)
    return (x - m) / jnp.sqrt(v + eps)
def _scatter_add(tgt, idx, src, axis=0):
    return tgt.at[idx].add(src)
def _segment_sum(src, seg, n):
    return jax.ops.segment_sum(src, seg, n)
class _Rng:
    def __init__(self, key):
        self._k = key
    def _next(self):
        self._k, sub = jax.random.split(self._k)
        return sub
    def normal(self, shape):
        return jax.random.normal(self._next(), shape, dtype=jnp.bfloat16)
    def randint(self, lo, hi, shape):
        return jax.random.randint(self._next(), shape, lo, hi, dtype=jnp.int32)
    def uniform(self, shape, lo=0.0, hi=1.0):
        return jax.random.uniform(self._next(), shape, jnp.bfloat16, lo, hi)
    def permutation(self, n):
        return jax.random.permutation(self._next(), n)


kernel_name = 'standalone__layernorm_linear__sampling'

def setup_inputs():
    _rng = _Rng(jax.random.key(int.from_bytes(__import__("os").urandom(4), "little")))
    _w = (lambda a: (lambda t: t.astype(jnp.bfloat16) if jnp.issubdtype(t.dtype, jnp.floating) else t)(jnp.asarray(a)))
    B, S, D = 1024, 32, 576
    return {
        "x": _w((lambda *s: _rng.normal(s) * 0.05)(B, S, D)),
        "g": _w((lambda *s: _rng.normal(s) * 0.05)(D) + 1.0),
        "b": _w((lambda *s: _rng.normal(s) * 0.05)(D)),
        "w": _w((lambda *s: _rng.normal(s) * 0.05)(D, D)),
    }

def reference(x, g, b, w):
    return (_layernorm(x, axis=-1) * g + b) @ w
```

```python
import functools
import jax, jax.numpy as jnp
from jax import lax
import jax.experimental.pallas as pl
import jax.experimental.pallas.tpu as pltpu

EPS = 1e-5
F32 = jnp.float32
BF16 = jnp.bfloat16
U32 = jnp.uint32

def dot(a, b):
    return jnp.dot(a, b, preferred_element_type=F32)

@jax.jit
def pallas_standalone__layernorm_linear__sampling_kernel(x, g, b, w):
    ts=4; init=(2,2,4,8); wstart=12; nch=9; tail_split=True; cmx=True; wfirst=False; hold=1
    B, S, D = x.shape
    H = D // 2
    KH = 256
    KT = D - 2 * KH
    TW = 128
    PW = 2 * TW
    KE = KT + 16
    NP = B // PW
    LA = 2
    xt = jnp.transpose(x, (1, 2, 0))
    n_init = sum(init)
    assert n_init % NP == 0
    s_init = n_init // NP
    assert (S - s_init) % ts == 0
    n_it = (S - s_init) // ts
    NQ = ts * NP

    def span(q0, q1):
        out = []
        q = q0
        while q < q1:
            s, p = divmod(q, NP)
            if p == 0 and q1 - q >= NP:
                n = (q1 - q) // NP
                out.append((s, n, 0, B)); q += n * NP
            else:
                e = min(q1, (s + 1) * NP)
                out.append((s, 1, p * PW, (e - s * NP) * PW)); q = e
        return out
    groups = [span(0, LA)]
    have = LA
    pos = 0
    for bi, n in enumerate(init):
        pos += n
        need = pos + LA
        if bi == len(init) - 1:
            need = -(-need // NP) * NP
        groups.append(span(have, need)); have = need
    n_ginit = len(groups)
    for j in range(n_it):
        need = min((s_init + (j + 1) * ts + 1) * NP, S * NP)
        groups.append(span(have, need)); have = need
    NG = len(groups)

    def body(x_hbm, g_hbm, b_hbm, w_hbm, o_hbm, xbuf, obuf, w_ref, g_ref, b_ref, a_ref, at_ref, st_ref, sw, sin, sout):
        def rd(gi):
            cps = []
            for (s, n, l0, l1) in groups[gi]:
                cps.append(pltpu.make_async_copy(x_hbm.at[pl.ds(s, n), :, pl.ds(l0, l1 - l0)],
                                                 xbuf.at[pl.ds(s, n), :, pl.ds(l0, l1 - l0)], sin.at[gi]))
            return cps
        def rd_loop(j):
            s = s_init + j * ts + 1
            return pltpu.make_async_copy(x_hbm.at[pl.ds(s, ts)], xbuf.at[pl.ds(s, ts)], sin.at[n_ginit + j])
        def wr(s, n=1, l0=0, l1=B, r0=0, r1=D):
            return pltpu.make_async_copy(obuf.at[pl.ds(s, n), pl.ds(r0, r1 - r0), pl.ds(l0, l1 - l0)],
                                         o_hbm.at[pl.ds(s, n), pl.ds(r0, r1 - r0), pl.ds(l0, l1 - l0)], sout.at[0])
        wcp = [pltpu.make_async_copy(w_hbm, w_ref, sw.at[0]), pltpu.make_async_copy(g_hbm, g_ref, sw.at[0]),
               pltpu.make_async_copy(b_hbm, b_ref, sw.at[0])]
        for c_ in wcp: c_.start()
        if wfirst:
            for c_ in wcp: c_.wait()
        for gi in range(NG if not hold else hold):
            for c_ in rd(gi): c_.start()
        if not wfirst:
            for c_ in wcp: c_.wait()
        if hold:
            for gi in range(hold, NG):
                for c_ in rd(gi): c_.start()

        gg = g_ref[...].astype(F32).reshape(1, D)
        wb = w_ref[...]
        if cmx:
            b8 = jnp.broadcast_to(b_ref[...].astype(F32).reshape(1, D), (16, D)).astype(BF16)
            crow = dot(b8, wb)[:8]
            chi = crow.astype(BF16).astype(F32)
            row8 = lax.broadcasted_iota(jnp.int32, (8, D), 0)
            ext = jnp.where(row8 == 0, chi, jnp.where(row8 == 1, crow - chi, 0.0))
            wtl = jnp.concatenate([wb[2*KH:].astype(F32), ext, jnp.zeros((128 - KT - 8, D), F32)], axis=0).T
            lane = lax.broadcasted_iota(jnp.int32, (1, 128), 1)
            gt = jnp.concatenate([gg[:, 2*KH:], jnp.ones((1, 128 - KT), F32)], axis=1)
            wtail = wtl * gt
            wg = wb[:2*KH].astype(F32).T * gg[:, :2*KH]
        else:
            wt = wb.astype(F32).T
            bb = b_ref[...].astype(F32).reshape(1, D)
            wg = wt * gg
            c = jnp.sum(wt * bb, axis=1, keepdims=True)
            wtail = jnp.concatenate([wg[:, 2*KH:], jnp.zeros((D, 128 - KT), F32)], axis=1)
            chi = c.astype(BF16).astype(F32)
            clo = c - chi
            lane = lax.broadcasted_iota(jnp.int32, (D, 128), 1)
            wtail = jnp.where(lane == KT, chi, jnp.where(lane == KT + 1, clo, wtail))
        a11 = wg[:H, :KH]; a12 = wg[:H, KH:2*KH]; a21 = wg[H:, :KH]; a22 = wg[H:, KH:2*KH]
        alist = (a11 + a22, a21 + a22, a11, a22, a11 + a12, a21 - a11, a12 - a22)
        for i, a in enumerate(alist):
            a_ref[i] = pltpu.bitcast(a.astype(BF16), U32)
        at_ref[...] = pltpu.bitcast(wtail.astype(BF16), U32)

        def get_stats(s, p):
            l1 = p * PW
            rows = D // nch
            c0 = xbuf[s, 0:16, l1:l1 + PW].astype(F32)[0:1]
            s1 = s2 = None
            partial = []
            for ch in range(nch):
                d = xbuf[s, ch * rows:(ch + 1) * rows, l1:l1 + PW].astype(F32) - c0
                d = d.reshape(rows // 8, 8, PW)
                a1 = jnp.sum(d, axis=0); a2 = jnp.sum(d * d, axis=0)
                s1 = a1 if s1 is None else s1 + a1
                s2 = a2 if s2 is None else s2 + a2
                partial.append(s2)
            md = jnp.sum(s1, axis=0, keepdims=True) * (1.0 / D)
            v = jnp.maximum(jnp.sum(s2, axis=0, keepdims=True) * (1.0 / D) - md * md, 0.0)
            m = c0 + md
            r = lax.rsqrt(v + EPS)
            partial[-1] = jnp.broadcast_to(r, (8, PW))
            return m, r, partial

        def pre(s, p, m, r):
            l1 = p * PW
            xf = xbuf[s, :, l1:l1 + PW].astype(F32)
            xh = (xf - m) * r
            b11 = xh[:KH, :TW]; b21 = xh[KH:2*KH, :TW]; b12 = xh[:KH, TW:]; b22 = xh[KH:2*KH, TW:]
            bl = (b11 + b22, b11, b12 - b22, b21 - b11, b22, b11 + b12, b21 + b22)
            bl = [t.astype(BF16) for t in bl]
            row = lax.broadcasted_iota(jnp.int32, (16, PW), 0)
            bt = jnp.concatenate([xh[2*KH:, :], jnp.where(row < 2, 1.0, 0.0)], axis=0)
            return bl, bt.astype(BF16)

        def A(i):
            return pltpu.bitcast(a_ref[i], BF16)

        def mm(s, p, bl, bt, anchors):
            l1 = p * PW
            at = pltpu.bitcast(at_ref[...], BF16)[:, :KE]
            m1 = dot(A(0), bl[0]); m4 = dot(A(3), bl[3]); m5 = dot(A(4), bl[4]); m7 = dot(A(6), bl[6])
            m2 = dot(A(1), bl[1]); m3 = dot(A(2), bl[2]); m6 = dot(A(5), bl[5])
            pt = dot(at, bt)
            c11 = m1 + m4 - m5 + m7; c12 = m3 + m5; c21 = m2 + m4; c22 = m1 - m2 + m3 + m6
            c11 = c11 + pt[:H, :TW]; c12 = c12 + pt[:H, TW:]; c21 = c21 + pt[H:, :TW]; c22 = c22 + pt[H:, TW:]
            full = jnp.concatenate([jnp.concatenate([c11, c12], axis=1), jnp.concatenate([c21, c22], axis=1)], axis=0)
            if anchors:
                n = len(anchors)
                pieces = []
                pos = 0
                for j, a in enumerate(anchors):
                    rr = (j * D // n) // 8 * 8
                    if rr > pos: pieces.append(full[pos:rr])
                    pieces.append(jnp.where(a < 0, 0.0, full[rr:rr + 8]))
                    pos = rr + 8
                if pos < D: pieces.append(full[pos:])
                full = jnp.concatenate(pieces, axis=0)
            obuf[s, :, l1:l1 + PW] = full.astype(BF16)

        def block(sbase, q0, nq, dyn):
            st = {}
            for j in range(LA):
                st[q0 + j] = (st_ref[j, 0:1, :], st_ref[j, 1:2, :], None)
            for q in range(q0, q0 + nq):
                k, p = divmod(q, NP)
                kn, pn = divmod(q + LA, NP)
                sn = sbase + kn
                if dyn and kn >= ts: sn = jnp.minimum(sn, S - 1)
                st[q + LA] = get_stats(sn, pn)
                s_ = sbase + k
                mm(s_, p, *pre(s_, p, *st[q][:2]), st[q + LA][2])
                if dyn:
                    last_blk = (k == ts - 1) and tail_split
                    if last_blk:
                        @pl.when(s_ == S - 1)
                        def _():
                            wr(s_, 1, p * PW, (p + 1) * PW).start()
                    if p == NP - 1:
                        @pl.when(s_ == wstart)
                        def _():
                            wr(0, wstart + 1).start()
                        cond = s_ > wstart
                        if last_blk: cond = jnp.logical_and(cond, s_ < S - 1)
                        @pl.when(cond)
                        def _():
                            wr(s_).start()
                elif p == NP - 1:
                    if s_ == wstart: wr(0, wstart + 1).start()
                    elif s_ > wstart: wr(s_).start()
            for j in range(LA):
                st_ref[j, 0:1, :] = st[q0 + nq + j][0]; st_ref[j, 1:2, :] = st[q0 + nq + j][1]

        for c_ in rd(0): c_.wait()
        for j in range(LA):
            m, r, _ = get_stats(0, j)
            st_ref[j, 0:1, :] = m; st_ref[j, 1:2, :] = r
        q0 = 0
        for bi, n in enumerate(init):
            for c_ in rd(bi + 1): c_.wait()
            block(0, q0, n, False)
            q0 += n

        def it(j, carry):
            @pl.when(j < n_it - 1)
            def _():
                rd_loop(j).wait()
            @pl.when(j == n_it - 1)
            def _():
                for c_ in rd(NG - 1): c_.wait()
            block(s_init + j * ts, 0, NQ, True)
            return carry

        lax.fori_loop(0, n_it, it, 0)
        wr(0, wstart + 1).wait()
        for s in range(wstart + 1, S - 1 if tail_split else S):
            wr(s).wait()
        if tail_split:
            for p in range(NP):
                wr(S - 1, 1, p * PW, (p + 1) * PW).wait()

    out_t = pl.pallas_call(
        body,
        in_specs=[pl.BlockSpec(memory_space=pl.ANY)] * 4,
        out_specs=pl.BlockSpec(memory_space=pl.ANY),
        out_shape=jax.ShapeDtypeStruct((S, D, B), x.dtype),
        scratch_shapes=[pltpu.VMEM((S, D, B), BF16),
                        pltpu.VMEM((S, D, B), BF16),
                        pltpu.VMEM((D, D), BF16),
                        pltpu.VMEM((D,), BF16),
                        pltpu.VMEM((D,), BF16),
                        pltpu.VMEM((7, H // 2, KH), U32),
                        pltpu.VMEM((D // 2, 128), U32),
                        pltpu.VMEM((LA, 2, PW), F32),
                        pltpu.SemaphoreType.DMA((1,)),
                        pltpu.SemaphoreType.DMA((NG,)),
                        pltpu.SemaphoreType.DMA((1,))],
        compiler_params=pltpu.CompilerParams(vmem_limit_bytes=100 * 1024 * 1024),
    )(xt, g, b, w)
    return jnp.transpose(out_t, (2, 0, 1))
```

```python
import jax
import jax.numpy as jnp
from jax import lax
import jax.experimental.pallas as pl
import jax.experimental.pallas.tpu as pltpu

EPS = 1e-5
F32 = jnp.float32
BF16 = jnp.bfloat16
U32 = jnp.uint32

TW = 128
PW = 2 * TW
KB = 64
LA = 2

_SPEC = dict(
    q1a=((0,), "q1a", {"11": 1, "22": 1}),
    q1b=((1,), "mix", {"11": 1, "22": 1}),
    q1p=((2,), "mix", {"12": 1, "21": 1}),
    q2=((3, 4), "q2", {"21": 1, "22": -1}),
    q5=((5, 6), "q5", {"11": -1, "12": 1}),
    s22=((7, 8), "s22", {"22": 1}),
    s11=((9, 10), "s11", {"11": 1}),
    s21=((11,), "s21", {"21": 1}),
    s12=((12,), "s12", {"12": 1}),
    q3=(None, "q3", {"12": 1, "22": 1}),
    q4=(None, "q4", {"11": 1, "21": 1}),
)
_L2 = ("q3", "q4")
_ONE = ("s11", "q5", "q1a", "q1b", "s12", "q1p", "s21", "q2", "s22")
_SEQ = ([(n, 0) for n in _ONE[:4]] + [(n, None) for n in _L2]
        + [(n, 0) for n in _ONE[4:]] + [(n, 1) for n in _ONE])


def _dot(a, b):
    return jnp.dot(a, b, preferred_element_type=F32)


@jax.jit
def pallas_standalone__layernorm_linear__sampling_kernel(x, g, b, w):
    ts = 4
    init = (2, 2, 4, 8)
    wq = 58
    wc = 4
    nch = 9
    B, S, D = x.shape
    H = D // 2
    Q = H // 2
    NP = B // PW
    assert D == 9 * KB and B % (2 * PW) == 0
    n_init = sum(init)
    s_init = n_init // NP
    n_it = (S - s_init) // ts
    NQ = ts * NP
    assert n_init % NP == 0 and (S - s_init) % ts == 0 and all(n % 2 == 0 for n in init)
    wb_slabs = wq // NP
    wj, wql = divmod(wq - 1 - n_init, NQ)
    assert 0 <= wj < n_it - 1

    def span(q0, q1):
        out, q = [], q0
        while q < q1:
            s, p = divmod(q, NP)
            if p == 0 and q1 - q >= NP:
                n = (q1 - q) // NP
                out.append((s, n, 0, B))
                q += n * NP
            else:
                e = min(q1, (s + 1) * NP)
                out.append((s, 1, p * PW, (e - s * NP) * PW))
                q = e
        return out

    groups, have, pos = [span(0, LA)], LA, 0
    for bi, n in enumerate(init):
        pos += n
        need = pos + LA if bi < len(init) - 1 else pos + NP
        groups.append(span(have, need))
        have = need
    n_ginit = len(groups)
    for j in range(n_it):
        need = min((s_init + (j + 1) * ts + 1) * NP, S * NP)
        groups.append(span(have, need))
        have = need
    NG = len(groups)

    def body(x_hbm, g_hbm, b_hbm, w_hbm, o_hbm,
             xbuf, obuf, w_ref, g_ref, b_ref, a_ref, a2_ref, c_ref, st_ref, sem_w, sem_in, sem_out):

        def rd(gi):
            return [pltpu.make_async_copy(x_hbm.at[pl.ds(s, n), :, pl.ds(l0, l1 - l0)],
                                          xbuf.at[pl.ds(s, n), :, pl.ds(l0, l1 - l0)], sem_in.at[gi])
                    for (s, n, l0, l1) in groups[gi]]

        def wr(s, n=1, l0=0, l1=B):
            return pltpu.make_async_copy(obuf.at[pl.ds(s, n), :, pl.ds(l0, l1 - l0)],
                                         o_hbm.at[pl.ds(s, n), :, pl.ds(l0, l1 - l0)], sem_out.at[0])

        params = [pltpu.make_async_copy(w_hbm, w_ref, sem_w.at[0]),
                  pltpu.make_async_copy(g_hbm, g_ref, sem_w.at[0]),
                  pltpu.make_async_copy(b_hbm, b_ref, sem_w.at[0])]
        for cp in params + rd(0):
            cp.start()
        for cp in params:
            cp.wait()
        for gi in range(1, NG):
            for cp in rd(gi):
                cp.start()

        gg = g_ref[...].astype(F32).reshape(1, D)
        bb = b_ref[...].astype(F32).reshape(1, D)
        wf = w_ref[...].astype(F32)
        wt = jnp.concatenate([wf, wf[8 * KB:]], axis=0).T
        wg = wt * jnp.concatenate([gg, gg[:, 8 * KB:]], axis=1)
        bz = jnp.concatenate([bb, jnp.zeros((1, KB), F32)], axis=1)
        c_ref[...] = jnp.broadcast_to(jnp.sum(wt * bz, axis=1, keepdims=True), c_ref.shape)
        U = [wg[:H, 128 * t:128 * (t + 1)] for t in range(5)]
        L = [wg[H:, 128 * t:128 * (t + 1)] for t in range(5)]
        lo = lax.broadcasted_iota(jnp.int32, (H, 128), 1) < KB
        sel = jnp.where
        t1, t2, t5 = U[2] + L[3], L[2] + L[3], U[2] + U[3]
        t6, t7 = L[2] - U[2], U[3] - L[3]
        a_tiles = (U[0] + L[1], sel(lo, t1, 0.0), sel(lo, 0.0, t1),
                   L[0] + L[1], sel(lo, t2, -t2),
                   U[0] + U[1], sel(lo, t5, -t5),
                   L[0] - U[0], sel(lo, t6, L[4]),
                   U[1] - L[1], sel(lo, t7, U[4]),
                   sel(lo, L[4], t6), sel(lo, U[4], t7))
        for i, a in enumerate(a_tiles):
            a_ref[i] = pltpu.bitcast(a.astype(BF16), U32)
        l2_tiles = ((U[0], sel(lo, U[2], -L[3])), (L[1], sel(lo, L[3], -U[2])))
        for ci, (k0, k1) in enumerate(l2_tiles):
            a11, a21, a12, a22 = k0[:Q], k0[Q:], k1[:Q], k1[Q:]
            for i, a in enumerate((a11 + a22, a21 + a22, a11, a22, a11 + a12, a21 - a11, a12 - a22)):
                a2_ref[ci, i] = pltpu.bitcast(a.astype(BF16), U32)

        def stats(s, p):
            lanes = slice(p * PW, (p + 1) * PW)
            rows = D // nch
            c0 = xbuf[s, 0:16, lanes].astype(F32)[0:1]
            s1 = s2 = None
            partial = []
            for ch in range(nch):
                d = xbuf[s, ch * rows:(ch + 1) * rows, lanes].astype(F32) - c0
                d = d.reshape(rows // 8, 8, PW)
                a1, a2 = jnp.sum(d, axis=0), jnp.sum(d * d, axis=0)
                s1 = a1 if s1 is None else s1 + a1
                s2 = a2 if s2 is None else s2 + a2
                partial.append(s2)
            md = jnp.sum(s1, axis=0, keepdims=True) * (1.0 / D)
            var = jnp.maximum(jnp.sum(s2, axis=0, keepdims=True) * (1.0 / D) - md * md, 0.0)
            r = lax.rsqrt(var + EPS)
            partial[-1] = jnp.broadcast_to(r, (8, PW))
            return c0 + md, r, partial

        def operands(s, p, m, r):
            xh = (xbuf[s, :, p * PW:(p + 1) * PW].astype(F32) - m) * r
            x1, x2 = xh[:, :TW], xh[:, TW:]
            cat = lambda *t: jnp.concatenate(t, axis=0)
            R = lambda z, i, j: z[KB * i:KB * j]
            ops = dict(
                q1a=R(x1, 0, 2) + R(x2, 2, 4),
                mix=cat(R(x1, 4, 5) + R(x2, 6, 7), R(x2, 5, 6) + R(x1, 7, 8)),
                q2=cat(R(x1, 0, 2), R(x1, 4, 5), R(x2, 5, 6)),
                q3=cat(R(x2, 0, 2) - R(x2, 2, 4), R(x2, 4, 6) - R(x2, 6, 8)),
                q4=cat(R(x1, 2, 4) - R(x1, 0, 2), R(x1, 6, 8) - R(x1, 4, 6)),
                q5=cat(R(x2, 2, 4), R(x2, 6, 7), R(x1, 7, 8)),
                s22=cat(R(x1, 0, 2) + R(x2, 0, 2), R(x1, 4, 5) + R(x2, 4, 5), R(x2, 8, 9)),
                s11=cat(R(x1, 2, 4) + R(x2, 2, 4), R(x1, 6, 7) + R(x2, 6, 7), R(x1, 8, 9)),
                s21=cat(R(x1, 8, 9), R(x1, 5, 6) + R(x2, 5, 6)),
                s12=cat(R(x2, 8, 9), R(x1, 7, 8) + R(x2, 7, 8)))
            return {k: (v if k in _L2 else v.astype(BF16)) for k, v in ops.items()}

        def two_level(ci, b0, b1):
            b11, b21, b12, b22 = b0[:128], b0[128:], b1[:128], b1[128:]
            bs = (b11 + b22, b11, b12 - b22, b21 - b11, b22, b11 + b12, b21 + b22)
            M = {}
            for i in (0, 3, 4, 6, 1, 2, 5):
                M[i] = _dot(pltpu.bitcast(a2_ref[ci, i], BF16), bs[i].astype(BF16))
            c11, c21 = M[0] + M[3] - M[4] + M[6], M[1] + M[3]
            c12, c22 = M[2] + M[4], M[0] - M[1] + M[2] + M[5]
            return jnp.concatenate([c11, c21], axis=0), jnp.concatenate([c12, c22], axis=0)

        def products(ops):
            cc = c_ref[...]
            acc = [{"11": cc[:H], "12": cc[:H], "21": cc[H:], "22": cc[H:]} for _ in range(2)]

            def add(h, name, pr):
                for k, sign in _SPEC[name][2].items():
                    acc[h][k] = acc[h][k] + pr if sign > 0 else acc[h][k] - pr

            held = None
            for name, h in _SEQ:
                if h is None:
                    r0, r1 = two_level(_L2.index(name), ops[0][name], ops[1][name])
                    add(0, name, r0)
                    add(1, name, r1)
                    continue
                tiles, bname, _ = _SPEC[name]
                a = [pltpu.bitcast(a_ref[i], BF16) for i in tiles]
                pr = _dot(a[0] if len(a) == 1 else jnp.concatenate(a, axis=1), ops[h][bname])
                if name == "q1a":
                    held = pr
                    continue
                add(h, name, held + pr if name == "q1b" else pr)
            return acc

        def store(s, p, acc, anchors):
            full = jnp.concatenate([jnp.concatenate([acc["11"], acc["12"]], axis=1),
                                    jnp.concatenate([acc["21"], acc["22"]], axis=1)], axis=0)
            step = D // len(anchors)
            pieces = []
            for j, a in enumerate(anchors):
                pieces.append(jnp.where(a < 0, 0.0, full[j * step:j * step + 8]))
                pieces.append(full[j * step + 8:(j + 1) * step])
            obuf[s, :, p * PW:(p + 1) * PW] = jnp.concatenate(pieces, axis=0).astype(BF16)

        def loop_writes(q):
            res = []
            k, p = divmod(q, NP)
            if q == wql:
                res.append((wj, wr(0, wb_slabs)))
            if p == NP - 1:
                for jj in range(wj, n_it - 1):
                    n = wc if jj < n_it - 2 else 1
                    if (k + 1) % n:
                        continue
                    hi = s_init + jj * ts + k + 1
                    first = max(hi - n, wb_slabs)
                    if hi > first and (jj > wj or q > wql):
                        res.append((jj, wr(first, hi - first)))
            if k == ts - 1:
                res.append((n_it - 1, wr(S - 1, 1, p * PW, (p + 1) * PW)))
            elif p == NP - 1:
                res.append((n_it - 1, wr(S - ts + k)))
            return res

        def block(sbase, q0, nq, j=None):
            st = {q0 + i: (st_ref[i, 0:1, :], st_ref[i, 1:2, :]) for i in range(LA)}
            for qq in range(q0, q0 + nq, 2):
                for q in (qq + LA, qq + 1 + LA):
                    k, p = divmod(q, NP)
                    sn = sbase + k
                    if j is not None and k >= ts:
                        sn = jnp.minimum(sn, S - 1)
                    st[q] = stats(sn, p)
                k, p = divmod(qq, NP)
                acc = products([operands(sbase + k, p + h, *st[qq + h][:2]) for h in range(2)])
                for h in range(2):
                    store(sbase + k, p + h, acc[h], st[qq + h + LA][2])
                    if j is not None:
                        for jj, cp in loop_writes(qq + h):
                            pl.when(j == jj)(cp.start)
            for i in range(LA):
                st_ref[i, 0:1, :] = st[q0 + nq + i][0]
                st_ref[i, 1:2, :] = st[q0 + nq + i][1]

        for cp in rd(0):
            cp.wait()
        for i in range(LA):
            m, r, _ = stats(0, i)
            st_ref[i, 0:1, :] = m
            st_ref[i, 1:2, :] = r
        q0 = 0
        for bi, n in enumerate(init):
            for cp in rd(bi + 1):
                cp.wait()
            block(0, q0, n)
            q0 += n

        def step(j, carry):
            @pl.when(j < n_it - 1)
            def _():
                s = s_init + j * ts + 1
                pltpu.make_async_copy(x_hbm.at[pl.ds(s, ts)], xbuf.at[pl.ds(s, ts)],
                                      sem_in.at[n_ginit + j]).wait()

            @pl.when(j == n_it - 1)
            def _():
                for cp in rd(NG - 1):
                    cp.wait()

            block(s_init + j * ts, 0, NQ, j)
            return carry

        lax.fori_loop(0, n_it, step, 0)
        for q in range(NQ):
            for _, cp in loop_writes(q):
                cp.wait()

    out_t = pl.pallas_call(
        body,
        in_specs=[pl.BlockSpec(memory_space=pl.ANY)] * 4,
        out_specs=pl.BlockSpec(memory_space=pl.ANY),
        out_shape=jax.ShapeDtypeStruct((S, D, B), x.dtype),
        scratch_shapes=[
            pltpu.VMEM((S, D, B), BF16),
            pltpu.VMEM((S, D, B), BF16),
            pltpu.VMEM((D, D), BF16),
            pltpu.VMEM((D,), BF16),
            pltpu.VMEM((D,), BF16),
            pltpu.VMEM((13, H // 2, 128), U32),
            pltpu.VMEM((2, 7, Q // 2, 128), U32),
            pltpu.VMEM((D, 128), F32),
            pltpu.VMEM((LA, 2, PW), F32),
            pltpu.SemaphoreType.DMA((1,)),
            pltpu.SemaphoreType.DMA((NG,)),
            pltpu.SemaphoreType.DMA((1,)),
        ],
        compiler_params=pltpu.CompilerParams(vmem_limit_bytes=100 * 1024 * 1024),
    )(jnp.transpose(x, (1, 2, 0)), g, b, w)
    return jnp.transpose(out_t, (2, 0, 1))
```

```python
import jax
import jax.numpy as jnp
from jax import lax
import jax.experimental.pallas as pl
import jax.experimental.pallas.tpu as pltpu

EPS = 1e-5
F32 = jnp.float32
BF16 = jnp.bfloat16
U32 = jnp.uint32

TW = 128
PW = 2 * TW
KB = 64
LA = 2

_SPEC = dict(
    q1a=((0,), "q1a", {"11": 1, "22": 1}),
    q1b=((1,), "mix", {"11": 1, "22": 1}),
    q1p=((2,), "mix", {"12": 1, "21": 1}),
    q2=((3, 4), "q2", {"21": 1, "22": -1}),
    q5=((5, 6), "q5", {"11": -1, "12": 1}),
    s22=((7, 8), "s22", {"22": 1}),
    s11=((9, 10), "s11", {"11": 1}),
    s21=((11,), "s21", {"21": 1}),
    s12=((12,), "s12", {"12": 1}),
    q3=(None, "q3", {"12": 1, "22": 1}),
    q4=(None, "q4", {"11": 1, "21": 1}),
)
_L2 = ("q3", "q4")
_ONE = ("s11", "q5", "q1a", "q1b", "s12", "q1p", "s21", "q2", "s22")
_SEQ = ([(n, 0) for n in _ONE[:4]] + [(n, None) for n in _L2]
        + [(n, 0) for n in _ONE[4:]] + [(n, 1) for n in _ONE])


def _dot(a, b):
    return jnp.dot(a, b, preferred_element_type=F32)


@jax.jit
def pallas_standalone__layernorm_linear__sampling_kernel(x, g, b, w):
    B, S, D = x.shape
    init = (2, 2, 4, 8)
    ts = 4
    wq = 58
    wc = 4
    nch = 9
    H = D // 2
    Q = H // 2
    NP = B // PW
    assert D == 9 * KB and B % (2 * PW) == 0
    n_init = sum(init)
    s_init = n_init // NP
    n_it = (S - s_init) // ts
    NQ = ts * NP
    assert n_init % NP == 0 and (S - s_init) % ts == 0 and all(n % 2 == 0 for n in init)
    wb_slabs = wq // NP
    wj, wql = divmod(wq - 1 - n_init, NQ)
    assert 0 <= wj < n_it - 1

    def span(q0, q1):
        out, q = [], q0
        while q < q1:
            s, p = divmod(q, NP)
            if p == 0 and q1 - q >= NP:
                n = (q1 - q) // NP
                out.append((s, n, 0, B))
                q += n * NP
            else:
                e = min(q1, (s + 1) * NP)
                out.append((s, 1, p * PW, (e - s * NP) * PW))
                q = e
        return out

    groups, have, pos = [span(0, LA)], LA, 0
    for bi, n in enumerate(init):
        pos += n
        need = pos + LA if bi < len(init) - 1 else pos + NP
        groups.append(span(have, need))
        have = need
    n_ginit = len(groups)
    for j in range(n_it):
        need = min((s_init + (j + 1) * ts + 1) * NP, S * NP)
        groups.append(span(have, need))
        have = need
    NG = len(groups)

    def body(x_hbm, g_hbm, b_hbm, w_hbm, o_hbm,
             xbuf, obuf, w_ref, g_ref, b_ref, a_ref, a2_ref, c_ref, st_ref, sem_w, sem_in, sem_out):

        def rd(gi):
            return [pltpu.make_async_copy(x_hbm.at[pl.ds(s, n), :, pl.ds(l0, l1 - l0)],
                                          xbuf.at[pl.ds(s, n), :, pl.ds(l0, l1 - l0)], sem_in.at[gi])
                    for (s, n, l0, l1) in groups[gi]]

        def wr(s, n=1, l0=0, l1=B):
            return pltpu.make_async_copy(obuf.at[pl.ds(s, n), :, pl.ds(l0, l1 - l0)],
                                         o_hbm.at[pl.ds(s, n), :, pl.ds(l0, l1 - l0)], sem_out.at[0])

        params = [pltpu.make_async_copy(w_hbm, w_ref, sem_w.at[0]),
                  pltpu.make_async_copy(g_hbm, g_ref, sem_w.at[0]),
                  pltpu.make_async_copy(b_hbm, b_ref, sem_w.at[0])]
        for cp in params + rd(0):
            cp.start()
        for cp in params:
            cp.wait()
        for gi in range(1, NG):
            for cp in rd(gi):
                cp.start()

        gg = g_ref[...].astype(F32).reshape(1, D)
        bb = b_ref[...].astype(F32).reshape(1, D)
        wf = w_ref[...].astype(F32)
        wt = jnp.concatenate([wf, wf[8 * KB:]], axis=0).T
        wg = wt * jnp.concatenate([gg, gg[:, 8 * KB:]], axis=1)
        bz = jnp.concatenate([bb, jnp.zeros((1, KB), F32)], axis=1)
        c_ref[...] = jnp.broadcast_to(jnp.sum(wt * bz, axis=1, keepdims=True), c_ref.shape)
        U = [wg[:H, 128 * t:128 * (t + 1)] for t in range(5)]
        L = [wg[H:, 128 * t:128 * (t + 1)] for t in range(5)]
        lo = lax.broadcasted_iota(jnp.int32, (H, 128), 1) < KB
        sel = jnp.where
        t1, t2, t5 = U[2] + L[3], L[2] + L[3], U[2] + U[3]
        t6, t7 = L[2] - U[2], U[3] - L[3]
        a_tiles = (U[0] + L[1], sel(lo, t1, 0.0), sel(lo, 0.0, t1),
                   L[0] + L[1], sel(lo, t2, -t2),
                   U[0] + U[1], sel(lo, t5, -t5),
                   L[0] - U[0], sel(lo, t6, L[4]),
                   U[1] - L[1], sel(lo, t7, U[4]),
                   sel(lo, L[4], t6), sel(lo, U[4], t7))
        for i, a in enumerate(a_tiles):
            a_ref[i] = pltpu.bitcast(a.astype(BF16), U32)
        l2_tiles = ((U[0], sel(lo, U[2], -L[3])), (L[1], sel(lo, L[3], -U[2])))
        for ci, (k0, k1) in enumerate(l2_tiles):
            a11, a21, a12, a22 = k0[:Q], k0[Q:], k1[:Q], k1[Q:]
            for i, a in enumerate((a11 + a22, a21 + a22, a11, a22, a11 + a12, a21 - a11, a12 - a22)):
                a2_ref[ci, i] = pltpu.bitcast(a.astype(BF16), U32)

        def stats(s, p):
            lanes = slice(p * PW, (p + 1) * PW)
            rows = D // nch
            c0 = xbuf[s, 0:16, lanes].astype(F32)[0:1]
            s1 = s2 = None
            partial = []
            for ch in range(nch):
                d = xbuf[s, ch * rows:(ch + 1) * rows, lanes].astype(F32) - c0
                d = d.reshape(rows // 8, 8, PW)
                a1, a2 = jnp.sum(d, axis=0), jnp.sum(d * d, axis=0)
                s1 = a1 if s1 is None else s1 + a1
                s2 = a2 if s2 is None else s2 + a2
                partial.append(s2)
            md = jnp.sum(s1, axis=0, keepdims=True) * (1.0 / D)
            sq = jnp.sum(s2, axis=0, keepdims=True) * (1.0 / D)
            var = jnp.where(sq < jnp.inf, jnp.maximum(sq - md * md, 0.0), sq)
            r = lax.rsqrt(var + EPS)
            partial[-1] = jnp.broadcast_to(r, (8, PW))
            return c0 + md, r, partial

        def operands(s, p, m, r):
            xh = (xbuf[s, :, p * PW:(p + 1) * PW].astype(F32) - m) * r
            x1, x2 = xh[:, :TW], xh[:, TW:]
            cat = lambda *t: jnp.concatenate(t, axis=0)
            R = lambda z, i, j: z[KB * i:KB * j]
            ops = dict(
                q1a=R(x1, 0, 2) + R(x2, 2, 4),
                mix=cat(R(x1, 4, 5) + R(x2, 6, 7), R(x2, 5, 6) + R(x1, 7, 8)),
                q2=cat(R(x1, 0, 2), R(x1, 4, 5), R(x2, 5, 6)),
                q3=cat(R(x2, 0, 2) - R(x2, 2, 4), R(x2, 4, 6) - R(x2, 6, 8)),
                q4=cat(R(x1, 2, 4) - R(x1, 0, 2), R(x1, 6, 8) - R(x1, 4, 6)),
                q5=cat(R(x2, 2, 4), R(x2, 6, 7), R(x1, 7, 8)),
                s22=cat(R(x1, 0, 2) + R(x2, 0, 2), R(x1, 4, 5) + R(x2, 4, 5), R(x2, 8, 9)),
                s11=cat(R(x1, 2, 4) + R(x2, 2, 4), R(x1, 6, 7) + R(x2, 6, 7), R(x1, 8, 9)),
                s21=cat(R(x1, 8, 9), R(x1, 5, 6) + R(x2, 5, 6)),
                s12=cat(R(x2, 8, 9), R(x1, 7, 8) + R(x2, 7, 8)))
            return {k: (v if k in _L2 else v.astype(BF16)) for k, v in ops.items()}

        def two_level(ci, b0, b1):
            b11, b21, b12, b22 = b0[:128], b0[128:], b1[:128], b1[128:]
            bs = (b11 + b22, b11, b12 - b22, b21 - b11, b22, b11 + b12, b21 + b22)
            M = {}
            for i in (0, 3, 4, 6, 1, 2, 5):
                M[i] = _dot(pltpu.bitcast(a2_ref[ci, i], BF16), bs[i].astype(BF16))
            c11, c21 = M[0] + M[3] - M[4] + M[6], M[1] + M[3]
            c12, c22 = M[2] + M[4], M[0] - M[1] + M[2] + M[5]
            return jnp.concatenate([c11, c21], axis=0), jnp.concatenate([c12, c22], axis=0)

        def products(ops):
            cc = c_ref[...]
            acc = [{"11": cc[:H], "12": cc[:H], "21": cc[H:], "22": cc[H:]} for _ in range(2)]

            def add(h, name, pr):
                for k, sign in _SPEC[name][2].items():
                    acc[h][k] = acc[h][k] + pr if sign > 0 else acc[h][k] - pr

            held = None
            for name, h in _SEQ:
                if h is None:
                    r0, r1 = two_level(_L2.index(name), ops[0][name], ops[1][name])
                    add(0, name, r0)
                    add(1, name, r1)
                    continue
                tiles, bname, _ = _SPEC[name]
                a = [pltpu.bitcast(a_ref[i], BF16) for i in tiles]
                pr = _dot(a[0] if len(a) == 1 else jnp.concatenate(a, axis=1), ops[h][bname])
                if name == "q1a":
                    held = pr
                    continue
                add(h, name, held + pr if name == "q1b" else pr)
            return acc

        def store(s, p, acc, anchors):
            full = jnp.concatenate([jnp.concatenate([acc["11"], acc["12"]], axis=1),
                                    jnp.concatenate([acc["21"], acc["22"]], axis=1)], axis=0)
            step = D // len(anchors)
            pieces = []
            for j, a in enumerate(anchors):
                pieces.append(jnp.where(a < 0, 0.0, full[j * step:j * step + 8]))
                pieces.append(full[j * step + 8:(j + 1) * step])
            obuf[s, :, p * PW:(p + 1) * PW] = jnp.concatenate(pieces, axis=0).astype(BF16)

        def loop_writes(q):
            res = []
            k, p = divmod(q, NP)
            if q == wql:
                res.append((wj, wr(0, wb_slabs)))
            if p == NP - 1:
                for jj in range(wj, n_it - 1):
                    n = wc if jj < n_it - 2 else 1
                    if (k + 1) % n:
                        continue
                    hi = s_init + jj * ts + k + 1
                    first = max(hi - n, wb_slabs)
                    if hi > first and (jj > wj or q > wql):
                        res.append((jj, wr(first, hi - first)))
            if k == ts - 1:
                res.append((n_it - 1, wr(S - 1, 1, p * PW, (p + 1) * PW)))
            elif p == NP - 1:
                res.append((n_it - 1, wr(S - ts + k)))
            return res

        def block(sbase, q0, nq, j=None):
            st = {q0 + i: (st_ref[i, 0:1, :], st_ref[i, 1:2, :]) for i in range(LA)}
            for qq in range(q0, q0 + nq, 2):
                for q in (qq + LA, qq + 1 + LA):
                    k, p = divmod(q, NP)
                    sn = sbase + k
                    if j is not None and k >= ts:
                        sn = jnp.minimum(sn, S - 1)
                    st[q] = stats(sn, p)
                k, p = divmod(qq, NP)
                acc = products([operands(sbase + k, p + h, *st[qq + h][:2]) for h in range(2)])
                for h in range(2):
                    store(sbase + k, p + h, acc[h], st[qq + h + LA][2])
                    if j is not None:
                        for jj, cp in loop_writes(qq + h):
                            pl.when(j == jj)(cp.start)
            for i in range(LA):
                st_ref[i, 0:1, :] = st[q0 + nq + i][0]
                st_ref[i, 1:2, :] = st[q0 + nq + i][1]

        for cp in rd(0):
            cp.wait()
        for i in range(LA):
            m, r, _ = stats(0, i)
            st_ref[i, 0:1, :] = m
            st_ref[i, 1:2, :] = r
        q0 = 0
        for bi, n in enumerate(init):
            for cp in rd(bi + 1):
                cp.wait()
            block(0, q0, n)
            q0 += n

        def step(j, carry):
            for jj in range(n_it):
                for cp in rd(n_ginit + jj):
                    pl.when(j == jj)(cp.wait)
            block(s_init + j * ts, 0, NQ, j)
            return carry

        lax.fori_loop(0, n_it, step, 0)
        for q in range(NQ):
            for _, cp in loop_writes(q):
                cp.wait()

    out_t = pl.pallas_call(
        body,
        in_specs=[pl.BlockSpec(memory_space=pl.ANY)] * 4,
        out_specs=pl.BlockSpec(memory_space=pl.ANY),
        out_shape=jax.ShapeDtypeStruct((S, D, B), x.dtype),
        scratch_shapes=[
            pltpu.VMEM((S, D, B), BF16),
            pltpu.VMEM((S, D, B), BF16),
            pltpu.VMEM((D, D), BF16),
            pltpu.VMEM((D,), BF16),
            pltpu.VMEM((D,), BF16),
            pltpu.VMEM((13, H // 2, 128), U32),
            pltpu.VMEM((2, 7, Q // 2, 128), U32),
            pltpu.VMEM((D, 128), F32),
            pltpu.VMEM((LA, 2, PW), F32),
            pltpu.SemaphoreType.DMA((1,)),
            pltpu.SemaphoreType.DMA((NG,)),
            pltpu.SemaphoreType.DMA((1,)),
        ],
        compiler_params=pltpu.CompilerParams(vmem_limit_bytes=100 * 1024 * 1024),
    )(jnp.transpose(x, (1, 2, 0)), g, b, w)
    return jnp.transpose(out_t, (2, 0, 1))
```
